```python
import os as _os
_os.environ.setdefault("JAX_PLATFORMS", "cpu")
import jax
import jax.numpy as jnp

def _softmax(x, axis=-1):
    return jax.nn.softmax(x, axis=axis)
def _gelu(x):
    return jax.nn.gelu(x, approximate=True)
def _silu(x):
    return jax.nn.silu(x)
def _sigmoid(x):
    return jax.nn.sigmoid(x)
def _layernorm(x, axis=-1, eps=1e-5):
    m = jnp.mean(x, axis=axis, keepdims=True)
    v = jnp.var(x, axis=axis, keepdims=True)
    return (x - m) / jnp.sqrt(v + eps)
def _scatter_add(tgt, idx, src, axis=0):
    return tgt.at[idx].add(src)
def _segment_sum(src, seg, n):
    return jax.ops.segment_sum(src, seg, n)
class _Rng:
    def __init__(self, key):
        self._k = key
    def _next(self):
        self._k, sub = jax.random.split(self._k)
        return sub
    def normal(self, shape):
        return jax.random.normal(self._next(), shape, dtype=jnp.bfloat16)
    def randint(self, lo, hi, shape):
        return jax.random.randint(self._next(), shape, lo, hi, dtype=jnp.int32)
    def uniform(self, shape, lo=0.0, hi=1.0):
        return jax.random.uniform(self._next(), shape, jnp.bfloat16, lo, hi)
    def permutation(self, n):
        return jax.random.permutation(self._next(), n)


kernel_name = 'parallel_sum__ssm_conv_h3__dense_activation_silu__prompt'

def setup_inputs():
    _rng = _Rng(jax.random.key(int.from_bytes(__import__("os").urandom(4), "little")))
    _w = (lambda a: (lambda t: t.astype(jnp.bfloat16) if jnp.issubdtype(t.dtype, jnp.floating) else t)(jnp.asarray(a)))
    def _A_setup():
        B, S, D = 1, 2048, 448
        ks = 4
        return {
            "q": _w((lambda *s: _rng.normal(s) * 0.05)(B, S, D)),
            "k": _w((lambda *s: _rng.normal(s) * 0.2)(B, S, D)),
            "v": _w((lambda *s: _rng.normal(s) * 0.2)(B, S, D)),
            "shift_k": _w((lambda *s: _rng.normal(s) * 0.2)(D, ks) * 0.5),
            "ssm_k": _w((lambda *s: _rng.normal(s) * 0.2)(D, S) * (1.0 / S ** 0.5)),
            "ssm_D": _w((lambda *s: _rng.normal(s) * 0.2)(D)),
        }
    _A_in = _A_setup()

    def _B_setup():
        B, S, D, F = 1, 2048, 448, 1792
        return {
            "x": _w((lambda *s: _rng.normal(s) * 0.05)(B, S, D)),
            "w1": _w((lambda *s: _rng.normal(s) * 0.05)(D, F) * (D ** -0.5)),
            "w2": _w((lambda *s: _rng.normal(s) * 0.05)(F, D) * (F ** -0.5)),
        }
    _B_in = _B_setup()

    return {
        "A_q": _A_in["q"],
        "A_k": _A_in["k"],
        "A_v": _A_in["v"],
        "A_shift_k": _A_in["shift_k"],
        "A_ssm_k": _A_in["ssm_k"],
        "A_ssm_D": _A_in["ssm_D"],
        "B_x": _B_in["x"],
        "B_w1": _B_in["w1"],
        "B_w2": _B_in["w2"],
    }

def reference(A_q, A_k, A_v, A_shift_k, A_ssm_k, A_ssm_D, B_x, B_w1, B_w2):
    def _A_ref(q, k, v, shift_k, ssm_k, ssm_D):
        B, S, D = q.shape
        ks = shift_k.shape[-1]
        k_pad = jnp.pad(k, ((0, 0), (ks - 1, 0), (0, 0)))
        k_shift = jnp.zeros_like(k)
        for t in range(ks):
            k_shift = k_shift + k_pad[:, t:t + S, :] * shift_k[:, ks - 1 - t][None, None, :]
        kv = k_shift * v
        L = 2 * S
        kv_pad = jnp.pad(kv, ((0, 0), (0, S), (0, 0)))
        kf_pad = jnp.pad(ssm_k, ((0, 0), (0, S)))
        kv_f = (lambda x, axes=(-2,-1): jnp.fft.rfft2(x.astype(jnp.float32), axes=axes))(kv_pad[:, None, :, :], axes=(1, 2))
        kf_f = (lambda x, axes=(-2,-1): jnp.fft.rfft2(x.astype(jnp.float32), axes=axes))(kf_pad[:, None, :], axes=(1, 2))
        kf_f = (lambda x, *d: x.transpose(*d))(kf_f, 1, 2, 0)
        y_f = kv_f * kf_f[None, :, :, :]
        y = (lambda x, s, axes=(-2,-1): jnp.fft.irfft2(x, s=s, axes=axes).astype(jnp.bfloat16))(y_f, (1, L), axes=(1, 2))[:, 0, :S, :]
        y = y + kv * ssm_D[None, None, :]
        return q * y

    def _B_ref(x, w1, w2):
        h = jnp.einsum("bsd,df->bsf", x, w1)
        h = _silu(h)
        out = jnp.einsum("bsf,fd->bsd", h, w2)
        return out

    x = A_q
    xn = _layernorm(x, axis=-1)
    return x + _A_ref(xn, A_k, A_v, A_shift_k, A_ssm_k, A_ssm_D) + _B_ref(xn, B_w1, B_w2)
```

```python
import functools

import numpy as np
import jax
import jax.numpy as jnp
import jax.experimental.pallas as pl
import jax.experimental.pallas.tpu as pltpu


C = 128
N2 = 2 * C
TM = 256
CPS = TM // C


def _dft_mats():
    f = np.arange(C, dtype=np.float64)[:, None] + 0.5
    t = np.arange(C, dtype=np.float64)[None, :]
    th = 2.0 * np.pi * f * t / N2
    fwd = np.concatenate([np.cos(th), -np.sin(th)], axis=0)
    tv = np.arange(C, 2 * C, dtype=np.float64)[:, None]
    fv = np.arange(C, dtype=np.float64)[None, :] + 0.5
    thv = 2.0 * np.pi * fv * tv / N2
    inv = np.concatenate([np.cos(thv), -np.sin(thv)], axis=1) * (2.0 / N2)
    return fwd, inv


def _kernel(q_ref, k_ref, v_ref, sk_ref, ssmk_ref, ssmd_ref, w1_ref, w2_ref,
            fwd_ref, inv_ref, o_ref,
            kbuf, kvf_re, kvf_im, kw_re, kw_im, kprev_re, kprev_im, zbuf):
    step = pl.program_id(0)
    D = q_ref.shape[-1]

    @pl.when(step == 0)
    def _():
        kbuf[0:8, :] = jnp.zeros((8, D), jnp.float32)
        kprev_re[...] = jnp.zeros(kprev_re.shape, jnp.float32)
        kprev_im[...] = jnp.zeros(kprev_im.shape, jnp.float32)

    x = q_ref[...].astype(jnp.float32)
    mu = jnp.mean(x, axis=-1, keepdims=True)
    xc = x - mu
    var = jnp.mean(xc * xc, axis=-1, keepdims=True)
    xn = xc * jax.lax.rsqrt(var + 1e-5)
    xn_b = xn.astype(jnp.bfloat16)

    kbuf[8:8 + TM, :] = k_ref[...].astype(jnp.float32)
    sk = sk_ref[...].astype(jnp.float32)
    ks = kbuf[8:8 + TM, :] * sk[0:1, :]
    for l in range(1, 4):
        ks = ks + kbuf[8 - l:8 - l + TM, :] * sk[l:l + 1, :]
    kbuf[0:8, :] = kbuf[TM:TM + 8, :]
    kv_b = (ks * v_ref[...].astype(jnp.float32)).astype(jnp.bfloat16)
    kv = kv_b.astype(jnp.float32)

    fwd = fwd_ref[...]
    inv = inv_ref[...]
    sgn = 1.0 - 2.0 * (jax.lax.broadcasted_iota(jnp.int32, (C, 1), 0) % 2).astype(jnp.float32)

    ys = []
    for c in range(CPS):
        m = step * CPS + c
        kvf = jnp.dot(fwd, kv_b[c * C:(c + 1) * C, :], preferred_element_type=jnp.float32)
        kvf_re[m] = kvf[:C]
        kvf_im[m] = kvf[C:]
        kf = jax.lax.dot_general(fwd, ssmk_ref[:, c * C:(c + 1) * C],
                                 (((1,), (1,)), ((), ())),
                                 preferred_element_type=jnp.float32)
        kre = kf[:C]
        kim = kf[C:]
        kw_re[m] = kprev_re[...] + sgn * kim
        kw_im[m] = kprev_im[...] - sgn * kre
        kprev_re[...] = kre
        kprev_im[...] = kim

        def body(j, carry):
            zr, zi = carry
            ar = kw_re[j]
            ai = kw_im[j]
            br = kvf_re[m - j]
            bi = kvf_im[m - j]
            zr = zr + (ar * br - ai * bi)
            zi = zi + (ar * bi + ai * br)
            return zr, zi

        z0 = jnp.zeros((C, D), jnp.float32)
        zr, zi = jax.lax.fori_loop(0, m + 1, body, (z0, z0))
        zbuf[0:C, :] = zr.astype(jnp.bfloat16)
        zbuf[C:N2, :] = zi.astype(jnp.bfloat16)
        ys.append(jnp.dot(inv, zbuf[...], preferred_element_type=jnp.float32))
    y = jnp.concatenate(ys, axis=0)

    h = jnp.dot(xn_b, w1_ref[...], preferred_element_type=jnp.float32)
    h = h * jax.nn.sigmoid(h)
    ffn = jnp.dot(h.astype(jnp.bfloat16), w2_ref[...], preferred_element_type=jnp.float32)

    ssmd = ssmd_ref[...].astype(jnp.float32)
    out = x + xn * (y + kv * ssmd) + ffn
    o_ref[...] = out.astype(o_ref.dtype)


@jax.jit
def pallas_parallel_sum__ssm_conv_h3__dense_activation_silu__prompt_kernel(
    A_q: jax.Array,
    A_k: jax.Array,
    A_v: jax.Array,
    A_shift_k: jax.Array,
    A_ssm_k: jax.Array,
    A_ssm_D: jax.Array,
    B_x: jax.Array,
    B_w1: jax.Array,
    B_w2: jax.Array,
):
    B, S, D = A_q.shape
    F = B_w1.shape[1]
    assert B == 1 and S % TM == 0
    n_chunks = S // C
    q = A_q.reshape(S, D)
    k = A_k.reshape(S, D)
    v = A_v.reshape(S, D)
    sk = A_shift_k.T
    ssmd = A_ssm_D.reshape(1, D)
    fwd_np, inv_np = _dft_mats()
    fwd = jnp.asarray(fwd_np, dtype=jnp.bfloat16)
    inv = jnp.asarray(inv_np, dtype=jnp.bfloat16)

    row = lambda i: (i, 0)
    const = lambda i: (0, 0)
    out = pl.pallas_call(
        _kernel,
        grid=(S // TM,),
        in_specs=[
            pl.BlockSpec((TM, D), row),
            pl.BlockSpec((TM, D), row),
            pl.BlockSpec((TM, D), row),
            pl.BlockSpec((4, D), const),
            pl.BlockSpec((D, TM), lambda i: (0, i)),
            pl.BlockSpec((1, D), const),
            pl.BlockSpec((D, F), const),
            pl.BlockSpec((F, D), const),
            pl.BlockSpec((N2, C), const),
            pl.BlockSpec((C, N2), const),
        ],
        out_specs=pl.BlockSpec((TM, D), row),
        out_shape=jax.ShapeDtypeStruct((S, D), A_q.dtype),
        scratch_shapes=[
            pltpu.VMEM((TM + 8, D), jnp.float32),
            pltpu.VMEM((n_chunks, C, D), jnp.float32),
            pltpu.VMEM((n_chunks, C, D), jnp.float32),
            pltpu.VMEM((n_chunks, C, D), jnp.float32),
            pltpu.VMEM((n_chunks, C, D), jnp.float32),
            pltpu.VMEM((C, D), jnp.float32),
            pltpu.VMEM((C, D), jnp.float32),
            pltpu.VMEM((N2, D), jnp.bfloat16),
        ],
        compiler_params=pltpu.CompilerParams(
            dimension_semantics=("arbitrary",),
            vmem_limit_bytes=96 * 1024 * 1024,
        ),
    )(q, k, v, sk, A_ssm_k, ssmd, B_w1, B_w2, fwd, inv)
    return out.reshape(B, S, D)
```

```python
import numpy as np
import jax
import jax.numpy as jnp
import jax.experimental.pallas as pl
import jax.experimental.pallas.tpu as pltpu


C = 128
N2 = 2 * C
TM = 256
NSTEP = 8
NCONV = 4
TO = 512
RS = 16
FFN_AT = 0


def _dft_mats():
    t = np.arange(C, dtype=np.float64)[:, None]
    f = np.arange(C, dtype=np.float64)[None, :] + 0.5
    th = 2.0 * np.pi * f * t / N2
    fwd = np.concatenate([np.cos(th), -np.sin(th)], axis=1)
    fv = np.arange(C, dtype=np.float64)[:, None] + 0.5
    tv = np.arange(C, 2 * C, dtype=np.float64)[None, :]
    thv = 2.0 * np.pi * fv * tv / N2
    inv = np.concatenate([np.cos(thv), -np.sin(thv)], axis=0) * (2.0 / N2)
    return fwd, inv


def _ln(q_ref):
    x = q_ref[...].astype(jnp.float32)
    mu = jnp.mean(x, axis=0, keepdims=True)
    xc = x - mu
    var = jnp.mean(xc * xc, axis=0, keepdims=True)
    xn = xc * jax.lax.rsqrt(var + 1e-5)
    return x, xn


def _ffn(xn, w1t, w2buf):
    h = jnp.dot(w1t[...], xn.astype(jnp.bfloat16), preferred_element_type=jnp.float32)
    h = h * jax.nn.sigmoid(h)
    return jnp.dot(w2buf[...], h.astype(jnp.bfloat16), preferred_element_type=jnp.float32)


def _conv(step, k_ref, v_ref, sk_ref, ssmk_ref, ssmd_ref, fwd_ref, inv_ref, ybuf, hook):
    DB, S = k_ref.shape
    NCH = S // C
    kf32 = k_ref[...].astype(jnp.float32)
    sk = sk_ref[...].astype(jnp.float32)
    lane = jax.lax.broadcasted_iota(jnp.int32, (DB, S), 1)
    ks = kf32 * sk[:, 0:1]
    for l in range(1, 4):
        sh = jnp.where(lane >= l, pltpu.roll(kf32, l, 1), 0.0)
        ks = ks + sh * sk[:, l:l + 1]
    kv_b = (ks * v_ref[...].astype(jnp.float32)).astype(jnp.bfloat16)
    kv = kv_b.astype(jnp.float32)
    fwd = fwd_ref[...]
    sgn = 1.0 - 2.0 * (jax.lax.broadcasted_iota(jnp.int32, (1, C), 1) % 2).astype(jnp.float32)
    kv_st = jnp.concatenate([kv_b[:, c * C:(c + 1) * C] for c in range(NCH)], axis=0)
    kvf = jnp.dot(kv_st, fwd, preferred_element_type=jnp.float32)
    ssmk = ssmk_ref[...]
    k_st = jnp.concatenate([ssmk[:, c * C:(c + 1) * C] for c in range(NCH)], axis=0)
    kf = jnp.dot(k_st, fwd, preferred_element_type=jnp.float32)
    zs = [[None] * (DB // RS) for _ in range(NCH)]
    for r in range(DB // RS):
        hook(r)
        def sl(a, c, im):
            return a[c * DB + r * RS:c * DB + (r + 1) * RS, (C if im else 0):(N2 if im else C)]
        kwr, kwi = [], []
        for c in range(NCH):
            if c == 0:
                kwr.append(sgn * sl(kf, c, 1)); kwi.append(-(sgn * sl(kf, c, 0)))
            else:
                kwr.append(sl(kf, c - 1, 0) + sgn * sl(kf, c, 1))
                kwi.append(sl(kf, c - 1, 1) - sgn * sl(kf, c, 0))
        for m in range(NCH):
            zr = zi = None
            for j in range(m + 1):
                br = sl(kvf, m - j, 0); bi = sl(kvf, m - j, 1)
                pr = kwr[j] * br - kwi[j] * bi
                pi = kwr[j] * bi + kwi[j] * br
                zr = pr if zr is None else zr + pr
                zi = pi if zi is None else zi + pi
            zs[m][r] = jnp.concatenate([zr, zi], axis=1).astype(jnp.bfloat16)
    z_st = jnp.concatenate([zs[m][r] for m in range(NCH) for r in range(DB // RS)], axis=0)
    y_st = jnp.dot(z_st, inv_ref[...], preferred_element_type=jnp.float32)
    ssmd = ssmd_ref[...].astype(jnp.float32)
    row0 = pl.multiple_of(step * DB, 8)
    per = TM // C
    for tb in range(NCH // per):
        yb = jnp.concatenate([y_st[(tb * per + i) * DB:(tb * per + i + 1) * DB, :]
                              for i in range(per)], axis=1)
        ybuf[tb, pl.ds(row0, DB), :] = yb + kv[:, tb * TM:(tb + 1) * TM] * ssmd


def _kernel(q_ref, k_ref, v_ref, sk_ref, ssmk_ref, ssmd_ref, w1_hbm, w2t_hbm,
            fwd_ref, inv_ref, o_ref, w1buf, w2buf, sems, w1t, abuf, xnbuf, ybuf):
    step = pl.program_id(0)
    cargs = (k_ref, v_ref, sk_ref, ssmk_ref, ssmd_ref, fwd_ref, inv_ref, ybuf)

    @pl.when(step == 0)
    def _():
        cp1 = pltpu.make_async_copy(w1_hbm, w1buf, sems.at[0])
        cp2 = pltpu.make_async_copy(w2t_hbm, w2buf, sems.at[1])
        cp1.start()
        cp2.start()
        _conv(step, *cargs, lambda r: None)
        cp1.wait()
        w1t[...] = w1buf[...].T
        cp2.wait()
        x, xn = _ln(q_ref)
        abuf[step] = x + _ffn(xn, w1t, w2buf)
        xnbuf[step] = xn

    @pl.when(jnp.logical_and(step > 0, step < NCONV))
    def _():
        x, xn = _ln(q_ref)
        st = {}

        def hook(r):
            if r == FFN_AT:
                st["f"] = _ffn(xn, w1t, w2buf)

        _conv(step, *cargs, hook)
        abuf[step] = x + st["f"]
        xnbuf[step] = xn

    @pl.when(step >= NCONV)
    def _():
        x, xn = _ln(q_ref)
        abuf[step] = x + _ffn(xn, w1t, w2buf)
        xnbuf[step] = xn
        per = TO // TM
        b = (step - NCONV) * per
        for i in range(per):
            o_ref[:, i * TM:(i + 1) * TM] = (
                abuf[b + i] + xnbuf[b + i] * ybuf[b + i]).astype(o_ref.dtype)


@jax.jit
def pallas_parallel_sum__ssm_conv_h3__dense_activation_silu__prompt_kernel(
    A_q: jax.Array,
    A_k: jax.Array,
    A_v: jax.Array,
    A_shift_k: jax.Array,
    A_ssm_k: jax.Array,
    A_ssm_D: jax.Array,
    B_x: jax.Array,
    B_w1: jax.Array,
    B_w2: jax.Array,
):
    B, S, D = A_q.shape
    F = B_w1.shape[1]
    assert B == 1 and S == NSTEP * TM and S == NCONV * TO and D % (16 * NCONV) == 0
    DB = D // NCONV
    qT = A_q.reshape(S, D).T
    kT = A_k.reshape(S, D).T
    vT = A_v.reshape(S, D).T
    w2T = B_w2.T
    ssmd = A_ssm_D.reshape(D, 1)
    fwd_np, inv_np = _dft_mats()
    fwd = jnp.asarray(fwd_np, dtype=jnp.bfloat16)
    inv = jnp.asarray(inv_np, dtype=jnp.bfloat16)
    cblk = lambda i: (jnp.minimum(i, NCONV - 1), 0)
    const = lambda i: (0, 0)
    out = pl.pallas_call(
        _kernel,
        grid=(NSTEP,),
        in_specs=[
            pl.BlockSpec((D, TM), lambda i: (0, i)),
            pl.BlockSpec((DB, S), cblk),
            pl.BlockSpec((DB, S), cblk),
            pl.BlockSpec((DB, 4), cblk),
            pl.BlockSpec((DB, S), cblk),
            pl.BlockSpec((DB, 1), cblk),
            pl.BlockSpec(memory_space=pl.ANY),
            pl.BlockSpec(memory_space=pl.ANY),
            pl.BlockSpec((C, N2), const),
            pl.BlockSpec((N2, C), const),
        ],
        out_specs=pl.BlockSpec((D, TO), lambda i: (0, jnp.maximum(i - NCONV, 0))),
        out_shape=jax.ShapeDtypeStruct((D, S), A_q.dtype),
        scratch_shapes=[
            pltpu.VMEM((D, F), jnp.bfloat16),
            pltpu.VMEM((D, F), jnp.bfloat16),
            pltpu.SemaphoreType.DMA((2,)),
            pltpu.VMEM((F, D), jnp.bfloat16),
            pltpu.VMEM((NSTEP, D, TM), jnp.float32),
            pltpu.VMEM((NSTEP, D, TM), jnp.float32),
            pltpu.VMEM((NSTEP, D, TM), jnp.float32),
        ],
        compiler_params=pltpu.CompilerParams(
            dimension_semantics=("arbitrary",),
            vmem_limit_bytes=100 * 1024 * 1024,
        ),
    )(qT, kT, vT, A_shift_k, A_ssm_k, ssmd, B_w1, w2T, fwd, inv)
    return out.T.reshape(B, S, D)
```
